```python
import os as _os
_os.environ.setdefault("JAX_PLATFORMS", "cpu")
import jax
import jax.numpy as jnp

def _softmax(x, axis=-1):
    return jax.nn.softmax(x, axis=axis)
def _gelu(x):
    return jax.nn.gelu(x, approximate=True)
def _silu(x):
    return jax.nn.silu(x)
def _sigmoid(x):
    return jax.nn.sigmoid(x)
def _layernorm(x, axis=-1, eps=1e-5):
    m = jnp.mean(x, axis=axis, keepdims=True)
    v = jnp.var(x, axis=axis, keepdims=True)
    return (x - m) / jnp.sqrt(v + eps)
def _scatter_add(tgt, idx, src, axis=0):
    return tgt.at[idx].add(src)
def _segment_sum(src, seg, n):
    return jax.ops.segment_sum(src, seg, n)
class _Rng:
    def __init__(self, key):
        self._k = key
    def _next(self):
        self._k, sub = jax.random.split(self._k)
        return sub
    def normal(self, shape):
        return jax.random.normal(self._next(), shape, dtype=jnp.bfloat16)
    def randint(self, lo, hi, shape):
        return jax.random.randint(self._next(), shape, lo, hi, dtype=jnp.int32)
    def uniform(self, shape, lo=0.0, hi=1.0):
        return jax.random.uniform(self._next(), shape, jnp.bfloat16, lo, hi)
    def permutation(self, n):
        return jax.random.permutation(self._next(), n)


kernel_name = 'gated_mix__ssm_conv_h3__mixer_s_mlp__prompt'

def setup_inputs():
    _rng = _Rng(jax.random.key(int.from_bytes(__import__("os").urandom(4), "little")))
    _w = (lambda a: (lambda t: t.astype(jnp.bfloat16) if jnp.issubdtype(t.dtype, jnp.floating) else t)(jnp.asarray(a)))
    def _A_setup():
        B, S, D = 1, 2048, 576
        ks = 4
        return {
            "q": _w((lambda *s: _rng.normal(s) * 0.05)(B, S, D)),
            "k": _w((lambda *s: _rng.normal(s) * 0.4)(B, S, D)),
            "v": _w((lambda *s: _rng.normal(s) * 0.4)(B, S, D)),
            "shift_k": _w((lambda *s: _rng.normal(s) * 0.4)(D, ks) * 0.5),
            "ssm_k": _w((lambda *s: _rng.normal(s) * 0.4)(D, S) * (1.0 / S ** 0.5)),
            "ssm_D": _w((lambda *s: _rng.normal(s) * 0.4)(D)),
        }
    _A_in = _A_setup()

    def _B_setup():
        B, S, D, F = 1, 2048, 576, 4608
        return {
            "x":  _w((lambda *s: _rng.normal(s) * 0.05)(B, S, D)),
            "w1": _w((lambda *s: _rng.normal(s) * 0.2)(D, D) * (D ** -0.5)),
            "w2": _w((lambda *s: _rng.normal(s) * 0.2)(D, D) * (D ** -0.5)),
            "w3": _w((lambda *s: _rng.normal(s) * 0.2)(D, F) * (D ** -0.5)),
            "w4": _w((lambda *s: _rng.normal(s) * 0.2)(F, D) * (F ** -0.5)),
        }
    _B_in = _B_setup()

    return {
        "A_q": _A_in["q"],
        "A_k": _A_in["k"],
        "A_v": _A_in["v"],
        "A_shift_k": _A_in["shift_k"],
        "A_ssm_k": _A_in["ssm_k"],
        "A_ssm_D": _A_in["ssm_D"],
        "B_x": _B_in["x"],
        "B_w1": _B_in["w1"],
        "B_w2": _B_in["w2"],
        "B_w3": _B_in["w3"],
        "B_w4": _B_in["w4"],
        "gate_w": _w((lambda *s: _rng.normal(s) * 0.05)(576) * 16.0),
    }

def reference(A_q, A_k, A_v, A_shift_k, A_ssm_k, A_ssm_D, B_x, B_w1, B_w2, B_w3, B_w4, gate_w):
    def _A_ref(q, k, v, shift_k, ssm_k, ssm_D):
        B, S, D = q.shape
        ks = shift_k.shape[-1]
        k_pad = jnp.pad(k, ((0, 0), (ks - 1, 0), (0, 0)))
        k_shift = jnp.zeros_like(k)
        for t in range(ks):
            k_shift = k_shift + k_pad[:, t:t + S, :] * shift_k[:, ks - 1 - t][None, None, :]
        kv = k_shift * v
        L = 2 * S
        kv_pad = jnp.pad(kv, ((0, 0), (0, S), (0, 0)))
        kf_pad = jnp.pad(ssm_k, ((0, 0), (0, S)))
        kv_f = (lambda x, axes=(-2,-1): jnp.fft.rfft2(x.astype(jnp.float32), axes=axes))(kv_pad[:, None, :, :], axes=(1, 2))
        kf_f = (lambda x, axes=(-2,-1): jnp.fft.rfft2(x.astype(jnp.float32), axes=axes))(kf_pad[:, None, :], axes=(1, 2))
        kf_f = (lambda x, *d: x.transpose(*d))(kf_f, 1, 2, 0)
        y_f = kv_f * kf_f[None, :, :, :]
        y = (lambda x, s, axes=(-2,-1): jnp.fft.irfft2(x, s=s, axes=axes).astype(jnp.bfloat16))(y_f, (1, L), axes=(1, 2))[:, 0, :S, :]
        y = y + kv * ssm_D[None, None, :]
        return q * y

    def _B_ref(x, w1, w2, w3, w4):
        B, S, D = x.shape
        h = _gelu(_layernorm(x, axis=-1) @ w1)
        c = D // 4
        g0 = jnp.pad(h[:, :, 0*c:1*c], ((0, 0), (1, 0), (0, 0)))[:, :S, :]
        g1 = jnp.pad(h[:, :, 1*c:2*c], ((0, 0), (0, 1), (0, 0)))[:, 1:, :]
        g2 = jnp.pad(h[:, :, 2*c:3*c], ((0, 0), (2, 0), (0, 0)))[:, :S, :]
        g3 = jnp.pad(h[:, :, 3*c:   ], ((0, 0), (0, 2), (0, 0)))[:, 2:, :]
        hs = jnp.concatenate([g0, g1, g2, g3], axis=-1) @ w2
        x1 = x + hs
        h2 = _gelu(_layernorm(x1, axis=-1) @ w3) @ w4
        return x1 + h2

    x = A_q
    g = _sigmoid((x * gate_w).sum(-1, keepdims=True))
    a = _A_ref(x, A_k, A_v, A_shift_k, A_ssm_k, A_ssm_D)
    b = _B_ref(x, B_w1, B_w2, B_w3, B_w4)
    return g * a + (1 - g) * b
```

```python
import contextlib
import numpy as np
import jax
import jax.numpy as jnp
from jax import lax
import jax.experimental.pallas as pl
import jax.experimental.pallas.tpu as pltpu

S, D, F = 2048, 576, 4608
C = 128
NC = S // C
G = D // 4
EPS = 1e-5
f32 = jnp.float32
bf16 = jnp.bfloat16


def _dft_mats():
    n = np.arange(C)[:, None].astype(np.float64)
    th = 2.0 * np.pi * (np.arange(C)[None, :] + 0.5) / (2 * C)
    ft = np.concatenate([np.cos(th * n), -np.sin(th * n)], axis=1)
    gt = ft.T / C
    return ft.astype(np.float32), gt.astype(np.float32)


def _gelu(x):
    c1 = 0.7978845608028654
    c2 = 0.7978845608028654 * 0.044715
    u = x * (c1 + c2 * (x * x))
    hx = 0.5 * x
    return hx + hx * jnp.tanh(u)


def _stats(x):
    m = jnp.mean(x, axis=0, keepdims=True)
    xc = x - m
    v = jnp.mean(xc * xc, axis=0, keepdims=True)
    return m, lax.rsqrt(v + EPS)


def _ln_cols(x):
    m = jnp.mean(x, axis=0, keepdims=True)
    xc = x - m
    v = jnp.mean(xc * xc, axis=0, keepdims=True)
    return xc * lax.rsqrt(v + EPS)


def _roll(x, s):
    u = pltpu.bitcast(x, jnp.uint32)
    return pltpu.bitcast(pltpu.roll(u, s, axis=1), bf16)


def _zero_like(x):
    u = pltpu.bitcast(x, jnp.uint32)
    u = lax.shift_right_logical(lax.shift_right_logical(u, jnp.uint32(16)), jnp.uint32(16))
    return pltpu.bitcast(u, f32)


def _dot(a, b):
    return jnp.dot(a, b, preferred_element_type=f32)


def _dot_nt(a, b):
    return lax.dot_general(a, b, (((1,), (1,)), ((), ())), preferred_element_type=f32)


def make_kernel(TM=256, TB=512, TF=512, RB=16, CU=1, CI=7, QW=1, PROF=0, PP=256, Z0=11, ODD=8, ORD=0):
    NSTEP = S // TM
    R = TM // C
    NB = S // TB
    NRB = D // RB
    if ODD < 0:
        bounds = list(range(PP, F, TF)) + [F]
    else:
        sizes = [TF] * (F // TF)
        sizes[ODD] -= PP
        bounds = [PP]
        for s_ in sizes:
            bounds.append(bounds[-1] + s_)
    NF = len(bounds) - 1

    def scope(name):
        return jax.named_scope(name) if PROF else contextlib.nullcontext()

    def kernel(q_hbm, k_hbm, v_hbm, sk_hbm, w1_hbm, w2_hbm, w3_hbm, w4_hbm,
               shift_hbm, dvec_hbm, gw_hbm, ft_hbm, gt_hbm,
               o_ref,
               q_v, k_v, v_v, sk_v, w1_v, w2_v, w3_v, w4_v,
               shift_v, dvec_v, gw_v, ft_v, gt_v,
               w1t, w2t, h_v, x1_v, xn2_v, g_v, par_v, U, H, Z, opq, sems, kv_sems):
        i = pl.program_id(0)

        def kv_copies(t):
            off = pl.multiple_of(t * TM, TM)
            return (pltpu.make_async_copy(k_hbm.at[:, pl.ds(off, TM)],
                                          k_v.at[:, pl.ds(off + C, TM)], kv_sems.at[0]),
                    pltpu.make_async_copy(v_hbm.at[:, pl.ds(off, TM)],
                                          v_v.at[:, pl.ds(off, TM)], kv_sems.at[1]))

        def w_copies(lo, n, s):
            return (pltpu.make_async_copy(w3_hbm.at[:, pl.ds(lo, n)], w3_v.at[:, pl.ds(lo, n)], sems.at[s]),
                    pltpu.make_async_copy(w4_hbm.at[:, pl.ds(lo, n)], w4_v.at[:, pl.ds(lo, n)], sems.at[s + 1]))

        def prologue():
            cp_w1 = pltpu.make_async_copy(w1_hbm, w1_v, sems.at[0])
            cp_w2 = pltpu.make_async_copy(w2_hbm, w2_v, sems.at[1])
            cp_sk = pltpu.make_async_copy(sk_hbm, sk_v, sems.at[2])
            cp_small = [pltpu.make_async_copy(s, d, sems.at[5 + n]) for n, (s, d) in enumerate(
                ((gw_hbm, gw_v), (shift_hbm, shift_v), (dvec_hbm, dvec_v), (ft_hbm, ft_v), (gt_hbm, gt_v)))]
            q0 = QW * TB
            cp_qa = pltpu.make_async_copy(q_hbm.at[:, pl.ds(0, q0)], q_v.at[:, pl.ds(0, q0)], sems.at[10])
            cp_qb = pltpu.make_async_copy(q_hbm.at[:, pl.ds(q0, S - q0)], q_v.at[:, pl.ds(q0, S - q0)],
                                          sems.at[11])
            cp_wa = w_copies(0, PP, 12) if PP else ()
            cp_wb = w_copies(PP, F - PP, 3)
            cp_w1.start()
            cp_qa.start()
            cp_qb.start()
            for c in cp_small:
                c.start()
            cp_w2.start()
            cp_sk.start()
            for c in cp_wa:
                c.start()
            for c in kv_copies(0):
                c.start()
            for c in cp_wb:
                c.start()

            h_v[:, 0:C] = jnp.zeros((D, C), bf16)
            h_v[:, C + S:] = jnp.zeros((D, C), bf16)
            k_v[:, 0:C] = jnp.zeros((D, C), bf16)
            Z[0:Z0] = jnp.zeros((Z0, D, 2 * C), f32)
            opq[0] = 0

            def stage_a(b):
                lo = b * TB
                acc = _dot(w1t[...], q_v[:, lo:lo + TB])
                for c in range(TB // C):
                    m, r = _stats(q_v[:, lo + c * C:lo + (c + 1) * C].astype(f32))
                    pre = (acc[:, c * C:(c + 1) * C] - par_v[6] * m) * r
                    h_v[:, C + lo + c * C:C + lo + (c + 1) * C] = _gelu(pre).astype(bf16)

            def stage_b(b):
                lo = b * TB
                parts = []
                for gi, sh in enumerate((1, -1, 2, -2)):
                    if sh > 0:
                        win = h_v[gi * G:(gi + 1) * G, lo:lo + TB + C]
                        parts.append(_roll(win, sh)[:, C:])
                    else:
                        win = h_v[gi * G:(gi + 1) * G, C + lo:C + lo + TB + C]
                        parts.append(_roll(win, TB + C + sh)[:, :TB])
                hs_in = jnp.concatenate(parts, axis=0)
                x = q_v[:, lo:lo + TB].astype(f32)
                x1 = x + _dot(w2t[...], hs_in)
                x1_v[:, lo:lo + TB] = x1
                xn2_v[lo:lo + TB, :] = _ln_cols(x1).astype(bf16).T

            acts = {}

            def pp_up(b):
                lo = b * TB
                acts[b] = _gelu(_dot(xn2_v[lo:lo + TB, :], w3_v[:, 0:PP])).astype(bf16)

            def pp_down(b):
                lo = b * TB
                x1_v[:, lo:lo + TB] = x1_v[:, lo:lo + TB] + _dot_nt(w4_v[:, 0:PP], acts.pop(b))

            lane = lax.broadcasted_iota(jnp.int32, (1, C), 1)
            sgn = (1 - 2 * (lane % 2)).astype(f32)
            prev = [None]
            hcount = [0]

            def stage_h(n):
                for _ in range(n):
                    j = hcount[0]
                    hcount[0] += 1
                    hj = _dot(sk_v[:, j * C:(j + 1) * C], ft_v[...])
                    hr, hi = hj[:, :C], hj[:, C:]
                    if prev[0] is None:
                        H[j, :, :C] = hr
                        H[j, :, C:] = hi
                    else:
                        H[j, :, :C] = hr - sgn * prev[0][1]
                        H[j, :, C:] = hi + sgn * prev[0][0]
                    prev[0] = (hr, hi)
                    zi = Z0 + (j - 4)
                    if j >= 4 and zi < NC - R:
                        Z[zi] = _zero_like(hj)

            with scope('wait1'):
                cp_w1.wait()
            w1 = w1_v[...]
            w1t[...] = w1.T
            s1 = jnp.sum(w1.astype(f32), axis=0, keepdims=True)
            par_v[6] = jnp.broadcast_to(s1, (C, D)).T
            with scope('wait1b'):
                cp_qa.wait()
            for b in range(QW):
                stage_a(b)
            with scope('wait2'):
                cp_qb.wait()
            for b in range(QW, NB):
                stage_a(b)
            with scope('wait3'):
                for c in cp_small:
                    c.wait()
                cp_w2.wait()
                cp_sk.wait()
                for c in cp_wa:
                    c.wait()
            w2t[...] = w2_v[...].T
            sh = shift_v[...].astype(f32)
            for j in range(4):
                par_v[j] = jnp.broadcast_to(sh[j:j + 1], (C, D)).T
            par_v[4] = jnp.broadcast_to(dvec_v[...].astype(f32).reshape(1, D), (C, D)).T
            par_v[5] = jnp.broadcast_to(gw_v[...].astype(f32).reshape(1, D), (C, D)).T
            stage_h(4)
            if PP:
                assert NB == 4
                stage_b(0)
                stage_h(2)
                stage_b(1)
                pp_up(0)
                stage_h(2)
                stage_b(2)
                pp_down(0)
                pp_up(1)
                stage_h(2)
                stage_b(3)
                pp_down(1)
                pp_up(2)
                stage_h(3)
                pp_down(2)
                pp_up(3)
                stage_h(3)
                pp_down(3)
            else:
                for b in range(NB):
                    stage_b(b)
                    stage_h((NC - 4) // NB)
            assert hcount[0] == NC
            with scope('wait4'):
                for c in cp_wb:
                    c.wait()

        with scope('prologue'):
            pl.when(i == 0)(prologue)

        base = pl.multiple_of(i * TM, TM)
        with scope('kvwait'):
            for c in kv_copies(i):
                c.wait()

        @pl.when(i + 1 < NSTEP)
        def _():
            for c in kv_copies(i + 1):
                c.start()

        kvs = []
        zero = opq[0]

        def conv_fwd():
            kwin = k_v[:, pl.ds(base, TM + C)]
            shifted = [kwin[:, C:]] + [_roll(kwin, j)[:, C:] for j in range(1, 4)]
            for a in range(R):
                off = pl.multiple_of(base + a * C, C)
                ks = shifted[0][:, a * C:(a + 1) * C].astype(f32) * par_v[0]
                for j in range(1, 4):
                    ks = ks + shifted[j][:, a * C:(a + 1) * C].astype(f32) * par_v[j]
                kv = (ks * v_v[:, pl.ds(off, C)].astype(f32)).astype(bf16)
                kvs.append(kv)
                U[zero + a] = _dot(kv, ft_v[...])

        def cmac(z, u, h):
            (ur, ui), (hr, hi) = u, h
            pr, pi = hr * ur - hi * ui, hr * ui + hi * ur
            return (pr, pi) if z is None else (z[0] + pr, z[1] + pi)

        def mac_one(r, rb):
            rs = slice(rb * RB, (rb + 1) * RB)
            z = (Z[r, rs, :C], Z[r, rs, C:]) if r < NC - R else None
            for b in range(R):
                if r - b >= 0:
                    z = cmac(z, (U[b, rs, :C], U[b, rs, C:]), (H[r - b, rs, :C], H[r - b, rs, C:]))
            dst = r - R if r >= R else NC - R + r
            Z[zero + dst, rs, :C] = z[0]
            Z[zero + dst, rs, C:] = z[1]

        def conv_mac(rb):
            for r in range(NC):
                mac_one(r, rb)

        pre = []

        def conv_inv():
            for a in range(R):
                off = pl.multiple_of(base + a * C, C)
                y = _dot(Z[NC - R + a].astype(bf16), gt_v[...])
                q = q_v[:, pl.ds(off, C)].astype(f32)
                g = jax.nn.sigmoid(jnp.sum(q * par_v[5], axis=0, keepdims=True))
                og = 1.0 - g
                ga = (g * q) * (y + kvs[a].astype(f32) * par_v[4])
                pre.append((ga + og * x1_v[:, pl.ds(off, C)], og))

        xn2 = xn2_v[pl.ds(base, TM), :]
        acc = None

        def up(c):
            return _dot(xn2, w3_v[:, bounds[c]:bounds[c + 1]])

        h3 = up(0)
        for c in range(NF):
            h3n = up(c + 1) if c + 1 < NF else None
            if c == CU:
                conv_fwd()
                for rb in range(NRB):
                    conv_mac(rb)
            if c == CI:
                conv_inv()
            act = _gelu(h3).astype(bf16)
            p = _dot_nt(w4_v[:, bounds[c]:bounds[c + 1]], act)
            acc = p if acc is None else acc + p
            h3 = h3n

        for a in range(R):
            pa, og = pre[a]
            o_ref[:, a * C:(a + 1) * C] = (pa + og * acc[:, a * C:(a + 1) * C]).astype(bf16)

    ft_np, gt_np = _dft_mats()

    def fn(A_q, A_k, A_v, A_shift_k, A_ssm_k, A_ssm_D, B_x, B_w1, B_w2, B_w3, B_w4, gate_w):
        qT = A_q[0].T
        kT = A_k[0].T
        vT = A_v[0].T
        hbm = pl.BlockSpec(memory_space=pltpu.MemorySpace.HBM)
        outT = pl.pallas_call(
            kernel,
            grid=(NSTEP,),
            in_specs=[hbm] * 13,
            out_specs=pl.BlockSpec((D, TM), lambda i: (0, i)),
            out_shape=jax.ShapeDtypeStruct((D, S), bf16),
            scratch_shapes=[
                pltpu.VMEM((D, S), bf16),
                pltpu.VMEM((D, C + S), bf16),
                pltpu.VMEM((D, S), bf16),
                pltpu.VMEM((D, S), bf16),
                pltpu.VMEM((D, D), bf16),
                pltpu.VMEM((D, D), bf16),
                pltpu.VMEM((D, F), bf16),
                pltpu.VMEM((D, F), bf16),
                pltpu.VMEM((4, D), bf16),
                pltpu.VMEM((D,), bf16),
                pltpu.VMEM((D,), bf16),
                pltpu.VMEM((C, 2 * C), bf16),
                pltpu.VMEM((2 * C, C), bf16),
                pltpu.VMEM((D, D), bf16),
                pltpu.VMEM((D, D), bf16),
                pltpu.VMEM((D, S + 2 * C), bf16),
                pltpu.VMEM((D, S), f32),
                pltpu.VMEM((S, D), bf16),
                pltpu.VMEM((8, C), f32),
                pltpu.VMEM((7, D, C), f32),
                pltpu.VMEM((R, D, 2 * C), f32),
                pltpu.VMEM((NC, D, 2 * C), f32),
                pltpu.VMEM((NC, D, 2 * C), f32),
                pltpu.SMEM((1,), jnp.int32),
                pltpu.SemaphoreType.DMA((14,)),
                pltpu.SemaphoreType.DMA((2,)),
            ],
            compiler_params=pltpu.CompilerParams(
                dimension_semantics=("arbitrary",),
                vmem_limit_bytes=110 * 1024 * 1024),
        )(qT, kT, vT, A_ssm_k, B_w1, B_w2, B_w3, B_w4.T,
          A_shift_k.T, A_ssm_D, gate_w,
          jnp.asarray(ft_np, bf16), jnp.asarray(gt_np, bf16))
        return outT.T[None]

    return jax.jit(fn)


_impl = make_kernel(PP=256, ODD=8)


@jax.jit
def pallas_gated_mix__ssm_conv_h3__mixer_s_mlp__prompt_kernel(
        A_q, A_k, A_v, A_shift_k, A_ssm_k, A_ssm_D, B_x, B_w1, B_w2, B_w3, B_w4, gate_w):
    return _impl(A_q, A_k, A_v, A_shift_k, A_ssm_k, A_ssm_D, B_x, B_w1, B_w2, B_w3, B_w4, gate_w)
```

```python
import contextlib
import numpy as np
import jax
import jax.numpy as jnp
from jax import lax
import jax.experimental.pallas as pl
import jax.experimental.pallas.tpu as pltpu

S, D, F = 2048, 576, 4608
C = 128
NC = S // C
G = D // 4
EPS = 1e-5
f32 = jnp.float32
bf16 = jnp.bfloat16
u32 = jnp.uint32


def _dft_mats():
    n = np.arange(C)[:, None].astype(np.float64)
    th = 2.0 * np.pi * (np.arange(C)[None, :] + 0.5) / (2 * C)
    ft = np.concatenate([np.cos(th * n), -np.sin(th * n)], axis=1)
    gt = ft.T / C
    return ft.astype(np.float32), gt.astype(np.float32)


def _gelu(x):
    c1 = 0.7978845608028654
    c2 = 0.7978845608028654 * 0.044715
    u = x * (c1 + c2 * (x * x))
    hx = 0.5 * x
    return hx + hx * jnp.tanh(u)


def _stats(x):
    m = jnp.mean(x, axis=0, keepdims=True)
    xc = x - m
    v = jnp.mean(xc * xc, axis=0, keepdims=True)
    return m, lax.rsqrt(v + EPS)


def _ln_cols(x):
    m = jnp.mean(x, axis=0, keepdims=True)
    xc = x - m
    v = jnp.mean(xc * xc, axis=0, keepdims=True)
    return xc * lax.rsqrt(v + EPS)


def _roll(x, s):
    return pltpu.bitcast(pltpu.roll(pltpu.bitcast(x, u32), s, axis=1), bf16)


def _dot(a, b):
    return jnp.dot(a, b, preferred_element_type=f32)


def _dot_nt(a, b):
    return lax.dot_general(a, b, (((1,), (1,)), ((), ())), preferred_element_type=f32)


SEQS = {
    0: "a b b u W4 d p4 b p1 u p1 d p2 b u d u W3 q3 h6 q3 h6 q2 h4 d",
    1: "a b b u W4 p1 d p4 b u d p3 b u d u W3 q8 h16 d",
    2: "a b b u W4 p1 d p4 b u d p3 b u d W3 q4 h8 u q4 h8 d",
    3: "a b b u W4 p1 d p4 b u d p3 b u W3 q4 h8 d u q4 h8 d",
}


def make_kernel(TM=256, TB=512, TF=512, RB=16, CU=0, CI=7, PROF=0, PP=256, SEQ=2, ZA=12,
                STRU=1, LA=1, UORD=2, GQ=1, DSPL=0, KV32=0):
    NSTEP = S // TM
    R = TM // C
    NB = S // TB
    NRB = D // RB
    bounds = list(range(PP, F, TF)) + [F]
    NF = len(bounds) - 1
    DH = D // 2
    TH = TM // 2
    NG = (F - PP) // (2 * TF)
    NFS = 2 * NG
    KH = TF // 2
    KU = 2 * C
    NP_ = NC - R

    def scope(name):
        return jax.named_scope(name) if PROF else contextlib.nullcontext()

    def kernel(q_hbm, k_hbm, v_hbm, sk_hbm, w1_hbm, w2_hbm, w3_hbm, w4_hbm,
               shift_hbm, dvec_hbm, gw_hbm, ft_hbm, gt_hbm,
               o_ref,
               q_v, k_v, v_v, qt_v, sk_v, w1_v, w2_v, w3_v, w4_v,
               shift_v, dvec_v, gw_v, ft_v, gt_v,
               w1t, w2t, h_v, x1_v, xn2_v, w3s, w4s, par_v, U, H, Z, opq, sems, kv_sems, *gbufs):
        i = pl.program_id(0)

        def kv_copies(t):
            off = pl.multiple_of(t * TM, TM)
            return (pltpu.make_async_copy(k_hbm.at[:, pl.ds(pl.multiple_of(off - C, C), TM + C)],
                                          k_v.at[t % 2], kv_sems.at[0]),
                    pltpu.make_async_copy(v_hbm.at[:, pl.ds(off, TM)], v_v.at[t % 2], kv_sems.at[1]))

        def w_copies(lo, n, s):
            return (pltpu.make_async_copy(w3_hbm.at[:, pl.ds(lo, n)], w3_v.at[:, pl.ds(lo, n)], sems.at[s]),
                    pltpu.make_async_copy(w4_hbm.at[:, pl.ds(lo, n)], w4_v.at[:, pl.ds(lo, n)], sems.at[s + 1]))

        def prologue():
            cp_w1 = pltpu.make_async_copy(w1_hbm, w1_v, sems.at[0])
            cp_w2 = pltpu.make_async_copy(w2_hbm, w2_v, sems.at[1])
            cp_sk = pltpu.make_async_copy(sk_hbm, sk_v, sems.at[2])
            cp_small = [pltpu.make_async_copy(s, d, sems.at[5 + n]) for n, (s, d) in enumerate(
                ((gw_hbm, gw_v), (shift_hbm, shift_v), (dvec_hbm, dvec_v), (ft_hbm, ft_v), (gt_hbm, gt_v)))]
            qcuts = [0, 256, 768, 1536, S]
            cp_q = [pltpu.make_async_copy(q_hbm.at[:, pl.ds(lo, hi - lo)], q_v.at[:, pl.ds(lo, hi - lo)],
                                          sems.at[(10, 11, 14, 15)[n]])
                    for n, (lo, hi) in enumerate(zip(qcuts[:-1], qcuts[1:]))]
            cp_wa = w_copies(0, PP, 12)
            cp_w3, cp_w4 = w_copies(PP, F - PP, 3)
            cp_w1.start()
            for c in cp_q:
                c.start()
            for c in cp_small:
                c.start()
            cp_w2.start()
            for c in cp_wa:
                c.start()
            cp_w4.start()
            cp_w3.start()
            cp_sk.start()
            cp_kv0 = (pltpu.make_async_copy(k_hbm.at[:, pl.ds(0, TM)], k_v.at[0, :, pl.ds(C, TM)],
                                            kv_sems.at[0]),
                      pltpu.make_async_copy(v_hbm.at[:, pl.ds(0, TM)], v_v.at[0], kv_sems.at[1]))
            for c in cp_kv0:
                c.start()
            cp_qt = [pltpu.make_async_copy(q_hbm.at[:, pl.ds(t * TM, TM)], qt_v.at[t], kv_sems.at[2])
                     for t in range(NSTEP)]

            h_v[:, 0:C] = jnp.zeros((D, C), bf16)
            h_v[:, C + S:] = jnp.zeros((D, C), bf16)
            k_v[0, :, 0:C] = jnp.zeros((D, C), bf16)
            Z[0:ZA] = jnp.zeros((ZA, D, 2 * C), f32)
            opq[0] = 0
            w3s[5, 0:8, 0:C] = jnp.zeros((8, C), u32)
            w4s[5, 0:8, 0:C] = jnp.zeros((8, C), u32)

            def stage_a(lo, n):
                if n % 512:
                    acc = jnp.concatenate([_dot(w1t[0:DH, :], q_v[:, lo:lo + n]),
                                           _dot(w1t[DH:, :], q_v[:, lo:lo + n])], axis=0)
                else:
                    acc = _dot(w1t[...], q_v[:, lo:lo + n])
                for c in range(n // C):
                    m, r = _stats(q_v[:, lo + c * C:lo + (c + 1) * C].astype(f32))
                    pre = (acc[:, c * C:(c + 1) * C] - par_v[6] * m) * r
                    h_v[:, C + lo + c * C:C + lo + (c + 1) * C] = _gelu(pre).astype(bf16)

            def stage_b(b):
                lo = b * TB
                parts = []
                for gi, sh in enumerate((1, -1, 2, -2)):
                    if sh > 0:
                        win = h_v[gi * G:(gi + 1) * G, lo:lo + TB + C]
                        parts.append(_roll(win, sh)[:, C:])
                    else:
                        win = h_v[gi * G:(gi + 1) * G, C + lo:C + lo + TB + C]
                        parts.append(_roll(win, TB + C + sh)[:, :TB])
                hs_in = jnp.concatenate(parts, axis=0)
                x = q_v[:, lo:lo + TB].astype(f32)
                x1 = x + _dot(w2t[...], hs_in)
                for t in range(TB // TM):
                    x1_v[lo // TM + t] = x1[:, t * TM:(t + 1) * TM]
                xn2_v[lo:lo + TB, :] = _ln_cols(x1).astype(bf16).T

            acts = {}

            def pp_up(b):
                lo = b * TB
                acts[b] = _gelu(_dot(xn2_v[lo:lo + TB, :], w3_v[:, 0:PP])).astype(bf16)

            def pp_down(b):
                lo = b * TB
                p = _dot_nt(w4_v[:, 0:PP], acts.pop(b))
                for t in range(TB // TM):
                    x1_v[lo // TM + t] = x1_v[lo // TM + t] + p[:, t * TM:(t + 1) * TM]

            def prep(src, dst, rh, c, lhs):
                lo = bounds[c]
                W_ = C * GQ
                for o in range(0, KH, W_):
                    for r in range(0, rh, 16):
                        t = dst[5, 0:8, 0:C]
                        if GQ > 1:
                            t = jnp.concatenate([t] * GQ, axis=1)
                        m11 = pltpu.bitcast(pltpu.bitcast(src[r:r + 16, lo + o:lo + o + W_], u32) | t,
                                            bf16).astype(f32)
                        m22 = pltpu.bitcast(pltpu.bitcast(
                            src[rh + r:rh + r + 16, lo + KH + o:lo + KH + o + W_], u32) | t, bf16).astype(f32)
                        m12 = src[r:r + 16, lo + KH + o:lo + KH + o + W_].astype(f32)
                        m21 = src[rh + r:rh + r + 16, lo + o:lo + o + W_].astype(f32)
                        if lhs:
                            ops = (m11 + m22, m21 + m22, m11 + m12, m21 - m11, m12 - m22)
                        else:
                            ops = (m11 + m22, m12 - m22, m21 - m11, m11 + m12, m21 + m22)
                        d0 = c * KH + o
                        for n, op in enumerate(ops):
                            dst[i + n, r // 2:r // 2 + 8, d0:d0 + W_] = pltpu.bitcast(op.astype(bf16), u32)

            def stage_h(j):
                H[j] = _dot(sk_v[:, j * C:(j + 1) * C], ft_v[...])

            with scope('wait1'):
                cp_w1.wait()
            w1t[...] = w1_v[...].T
            Z[ZA:NP_ + 1] = jnp.zeros((NP_ + 1 - ZA, D, 2 * C), f32)
            for n, (lo, hi) in enumerate(zip(qcuts[:-2], qcuts[1:-1])):
                with scope('waitq%d' % n):
                    cp_q[n].wait()
                if n == 0:
                    s1 = jnp.sum(w1_v[...].astype(f32), axis=0, keepdims=True)
                    par_v[6] = jnp.broadcast_to(s1, (C, D)).T
                while lo < hi:
                    n_ = (hi - lo) % 512 or 512
                    stage_a(lo, n_)
                    lo += n_
            with scope('wait3'):
                for c in cp_small:
                    c.wait()
                cp_w2.wait()
                cp_q[-1].wait()
                for c in cp_wa:
                    c.wait()
            for c in cp_qt:
                c.start()
            w2t[...] = w2_v[...].T
            sh = shift_v[...].astype(f32)
            for j in range(4):
                par_v[j] = jnp.broadcast_to(sh[j:j + 1], (C, D)).T
            par_v[4] = jnp.broadcast_to(dvec_v[...].astype(f32).reshape(1, D), (C, D)).T
            par_v[5] = jnp.broadcast_to(gw_v[...].astype(f32).reshape(1, D), (C, D)).T
            cnt = dict(a=0, b=0, u=0, d=0, h=0, p=0, q=0)
            fns = dict(a=lambda _: stage_a(qcuts[-2], S - qcuts[-2]), b=stage_b, u=pp_up, d=pp_down, h=stage_h,
                       p=lambda c: prep(w4_v, w4s, DH, c, True),
                       q=lambda c: prep(w3_v, w3s, KU, c, False))
            for tok in SEQS[SEQ].split():
                if tok == 'W4':
                    with scope('waitw4'):
                        cp_w4.wait()
                elif tok == 'W3':
                    with scope('waitw3'):
                        cp_w3.wait()
                        cp_sk.wait()
                else:
                    for _ in range(int(tok[1:] or 1)):
                        fns[tok[0]](cnt[tok[0]])
                        cnt[tok[0]] += 1
            with scope('waitend'):
                for c in list(cp_kv0) + cp_qt:
                    c.wait()
            assert cnt['h'] == NC and cnt['p'] == NFS and cnt['q'] == (NFS if STRU else 0), cnt

        with scope('prologue'):
            pl.when(i == 0)(prologue)

        base = pl.multiple_of(i * TM, TM)
        with scope('kvwait'):
            @pl.when(i > 0)
            def _():
                for c in kv_copies(i):
                    c.wait()

        @pl.when(i + 1 < NSTEP)
        def _():
            for c in kv_copies(i + 1):
                c.start()

        slot = i % 2

        kvs = []
        zero = opq[0]

        def conv_fwd():
            kwin = k_v[slot]
            shifted = [kwin[:, C:]] + [_roll(kwin, j)[:, C:] for j in range(1, 4)]
            for a in range(R):
                ks = shifted[0][:, a * C:(a + 1) * C].astype(f32) * par_v[0]
                for j in range(1, 4):
                    ks = ks + shifted[j][:, a * C:(a + 1) * C].astype(f32) * par_v[j]
                kv = ks * v_v[slot, :, a * C:(a + 1) * C].astype(f32)
                if KV32:
                    kvs.append(kv * par_v[4])
                    U[zero + a] = _dot(kv.astype(bf16), ft_v[...])
                else:
                    kv = kv.astype(bf16)
                    kvs.append(kv)
                    U[zero + a] = _dot(kv, ft_v[...])

        def cmac(z, u, h):
            (ur, ui), (hr, hi) = u, h
            pr, pi = hr * ur - hi * ui, hr * ui + hi * ur
            return (pr, pi) if z is None else (z[0] + pr, z[1] + pi)

        lane = lax.broadcasted_iota(jnp.int32, (1, C), 1)
        sgn = (1 - 2 * (lane % 2)).astype(f32)

        def mac_one(r, rs):
            z = (Z[r, rs, :C], Z[r, rs, C:]) if r < NP_ else None
            for b in range(R):
                if r - b >= 0:
                    z = cmac(z, (U[b, rs, :C], U[b, rs, C:]), (H[r - b, rs, :C], H[r - b, rs, C:]))
            return z

        def put(dst, rs, z):
            Z[zero + dst, rs, :C] = z[0]
            Z[zero + dst, rs, C:] = z[1]

        def conv_mac(rb):
            rs = slice(rb * RB, (rb + 1) * RB)
            yp = (Z[NP_, rs, :C], Z[NP_, rs, C:])
            for r in range(R):
                y = mac_one(r, rs)
                put(NP_ + 1 + r, rs, (y[0] - sgn * yp[1], y[1] + sgn * yp[0]))
                yp = y
            put(NP_, rs, yp)
            for r in range(R, NC):
                put(r - R, rs, mac_one(r, rs))

        pre = []

        def conv_inv():
            for a in range(R):
                y = _dot(Z[NP_ + 1 + a].astype(bf16), gt_v[...])
                q = qt_v[i, :, a * C:(a + 1) * C].astype(f32)
                g = jax.nn.sigmoid(jnp.sum(q * par_v[5], axis=0, keepdims=True))
                og = 1.0 - g
                ga = (g * q) * (y + (kvs[a] if KV32 else kvs[a].astype(f32) * par_v[4]))
                pre.append((ga + og * x1_v[i, :, a * C:(a + 1) * C], og))

        xn2 = xn2_v[pl.ds(base, TM), :]
        if STRU:
            a11, a12, a21, a22 = xn2[:TH, :KU], xn2[:TH, KU:2 * KU], xn2[TH:, :KU], xn2[TH:, KU:2 * KU]
            f11, f12, f21, f22 = (t.astype(f32) for t in (a11, a12, a21, a22))
            xa = [(f11 + f22).astype(bf16), (f21 + f22).astype(bf16), a11, a22,
                  (f11 + f12).astype(bf16), (f21 - f11).astype(bf16), (f12 - f22).astype(bf16)]
            xt = xn2[:, 2 * KU:]

        def up(c):
            lo, hi = bounds[c], bounds[c + 1]
            if c >= NFS or not STRU:
                h = _dot(xn2, w3_v[:, lo:hi])
                if c >= NFS:
                    return h
                return h[:TH, :KH], h[:TH, KH:], h[TH:, :KH], h[TH:, KH:]

            def bop(n):
                if n == 1:
                    return w3_v[0:KU, lo:lo + KH]
                if n == 4:
                    return w3_v[KU:2 * KU, lo + KH:hi]
                return pltpu.bitcast(w3s[{0: 0, 2: 1, 3: 2, 5: 3, 6: 4}[n], :, c * KH:(c + 1) * KH], bf16)

            m = {}
            order = {0: ('t', 3, 1, 2, 4, 0, 6, 5), 1: (3, 1, 2, 4, 0, 6, 5, 't'), 2: (3, 1, 't', 2, 4, 0, 6, 5)}[UORD]
            for n in order:
                m[n] = _dot(xt, w3_v[2 * KU:, lo:hi]) if n == 't' else _dot(xa[n], bop(n))
            t = m['t']
            c21 = (t[TH:, :KH] + m[3]) + m[1]
            c12 = (t[:TH, KH:] + m[2]) + m[4]
            c11 = (((t[:TH, :KH] + m[3]) - m[4]) + m[0]) + m[6]
            c22 = (((t[TH:, KH:] - m[1]) + m[2]) + m[0]) + m[5]
            return c11, c12, c21, c22

        tail = {}

        def act(c, h3):
            if c >= NFS:
                tail[c] = _gelu(h3).astype(bf16)
                return
            cs = slice((c % 2) * KH, (c % 2 + 1) * KH)
            c11, c12, c21, c22 = h3
            gb = gbufs[c // 2]
            gb[zero + 0, TH:, cs] = _gelu(c21)
            gb[zero + 1, :TH, cs] = _gelu(c12)
            gb[zero + 0, :TH, cs] = _gelu(c11)
            gb[zero + 1, TH:, cs] = _gelu(c22)

        accs = [None] * 7
        extra = []

        def down(g, ns):
            gb = gbufs[g]
            b11, b12, b21, b22 = (lambda: gb[0, :TH]), (lambda: gb[0, TH:]), (lambda: gb[1, :TH]), (lambda: gb[1, TH:])
            tf = (lambda: b11() + b22(), b11, lambda: b12() - b22(), lambda: b21() - b11(), b22,
                  lambda: b11() + b12(), lambda: b21() + b22())

            def aop(n):
                if n in (2, 3):
                    rows = slice(0, DH) if n == 2 else slice(DH, D)
                    o = 0 if n == 2 else KH
                    return jnp.concatenate([w4_v[rows, bounds[cc] + o:bounds[cc] + o + KH]
                                            for cc in (2 * g, 2 * g + 1)], axis=1)
                return pltpu.bitcast(w4s[{0: 0, 1: 1, 4: 2, 5: 3, 6: 4}[n], :, g * TF:(g + 1) * TF], bf16)

            for n in ns:
                m = _dot_nt(aop(n), tf[n]().astype(bf16))
                accs[n] = m if accs[n] is None else accs[n] + m

        h3s = {c: up(c) for c in range(LA)}
        for c in range(NF):
            if c + LA < NF:
                h3s[c + LA] = up(c + LA)
            if c == CU:
                conv_fwd()
                for rb in range(NRB):
                    conv_mac(rb)
            if c == CI:
                conv_inv()
            act(c, h3s.pop(c))
            if DSPL and c >= 2 and c % 2 == 0:
                down(c // 2 - 1, range(DSPL, 7))
            if c >= NFS:
                extra.append(_dot_nt(w4_v[:, bounds[c]:bounds[c + 1]], tail.pop(c)))
            elif c % 2 == 1:
                down(c // 2, range(DSPL) if DSPL else range(7))

        m1, m2, m3, m4, m5, m6, m7 = accs
        acc = jnp.concatenate([
            jnp.concatenate([m1 + m4 - m5 + m7, m3 + m5], axis=1),
            jnp.concatenate([m2 + m4, m1 - m2 + m3 + m6], axis=1)], axis=0)
        for e in extra:
            acc = acc + e

        for a in range(R):
            pa, og = pre[a]
            o_ref[:, a * C:(a + 1) * C] = (pa + og * acc[:, a * C:(a + 1) * C]).astype(bf16)

    ft_np, gt_np = _dft_mats()

    def fn(A_q, A_k, A_v, A_shift_k, A_ssm_k, A_ssm_D, B_x, B_w1, B_w2, B_w3, B_w4, gate_w):
        qT = A_q[0].T
        kT = A_k[0].T
        vT = A_v[0].T
        hbm = pl.BlockSpec(memory_space=pltpu.MemorySpace.HBM)
        outT = pl.pallas_call(
            kernel,
            grid=(NSTEP,),
            in_specs=[hbm] * 13,
            out_specs=pl.BlockSpec((D, TM), lambda i: (0, i)),
            out_shape=jax.ShapeDtypeStruct((D, S), bf16),
            scratch_shapes=[
                pltpu.VMEM((D, S), bf16),
                pltpu.VMEM((2, D, C + TM), bf16),
                pltpu.VMEM((2, D, TM), bf16),
                pltpu.VMEM((NSTEP, D, TM), bf16),
                pltpu.VMEM((D, S), bf16),
                pltpu.VMEM((D, D), bf16),
                pltpu.VMEM((D, D), bf16),
                pltpu.VMEM((D, F), bf16),
                pltpu.VMEM((D, F), bf16),
                pltpu.VMEM((4, D), bf16),
                pltpu.VMEM((D,), bf16),
                pltpu.VMEM((D,), bf16),
                pltpu.VMEM((C, 2 * C), bf16),
                pltpu.VMEM((2 * C, C), bf16),
                pltpu.VMEM((D, D), bf16),
                pltpu.VMEM((D, D), bf16),
                pltpu.VMEM((D, S + 2 * C), bf16),
                pltpu.VMEM((NSTEP, D, TM), f32),
                pltpu.VMEM((S, D), bf16),
                pltpu.VMEM((6, KU // 2, NFS * KH), u32),
                pltpu.VMEM((6, DH // 2, NFS * KH), u32),
                pltpu.VMEM((7, D, C), f32),
                pltpu.VMEM((R, D, 2 * C), f32),
                pltpu.VMEM((NC, D, 2 * C), f32),
                pltpu.VMEM((NC + 1, D, 2 * C), f32),
                pltpu.SMEM((1,), jnp.int32),
                pltpu.SemaphoreType.DMA((16,)),
                pltpu.SemaphoreType.DMA((3,)),
            ] + [pltpu.VMEM((2, TM, TF), f32)] * NG,
            compiler_params=pltpu.CompilerParams(
                dimension_semantics=("arbitrary",),
                vmem_limit_bytes=110 * 1024 * 1024),
        )(qT, kT, vT, A_ssm_k, B_w1, B_w2, B_w3, B_w4.T,
          A_shift_k.T, A_ssm_D, gate_w,
          jnp.asarray(ft_np, bf16), jnp.asarray(gt_np, bf16))
        return outT.T[None]

    return jax.jit(fn)


_impl = make_kernel(SEQ=2)


@jax.jit
def pallas_gated_mix__ssm_conv_h3__mixer_s_mlp__prompt_kernel(
        A_q, A_k, A_v, A_shift_k, A_ssm_k, A_ssm_D, B_x, B_w1, B_w2, B_w3, B_w4, gate_w):
    return _impl(A_q, A_k, A_v, A_shift_k, A_ssm_k, A_ssm_D, B_x, B_w1, B_w2, B_w3, B_w4, gate_w)
```

```python
import numpy as np
import jax
import jax.numpy as jnp
from jax import lax
import jax.experimental.pallas as pl
import jax.experimental.pallas.tpu as pltpu

S, D, F = 2048, 576, 4608
C = 128
NC = S // C
G = D // 4
EPS = 1e-5
f32 = jnp.float32
bf16 = jnp.bfloat16
u32 = jnp.uint32

TM = 256
TB = 512
TF = 512
PP = 256
RB = 16
ZA = 13
NSTEP = S // TM
R = TM // C
NRB = D // RB
BOUNDS = list(range(PP, F, TF)) + [F]
NF = len(BOUNDS) - 1
DH = D // 2
TH = TM // 2
NG = (F - PP) // (2 * TF)
NFS = 2 * NG
KH = TF // 2
KU = 2 * C
NP_ = NC - R
QCUTS = [0, 256, 768, 1536, S]
SEQ = "a b b u W4 p1 d p3 b u p1 d p3 b u d W3 q4 h8 u q4 h8 d"
UP_ORDER = (2, 't', 4, 3, 1, 0, 6, 5)
DOWN_ORDER = (1, 3, 2, 4, 0, 6, 5)
CI = 7


def _dft_mats():
    n = np.arange(C)[:, None].astype(np.float64)
    th = 2.0 * np.pi * (np.arange(C)[None, :] + 0.5) / (2 * C)
    ft = np.concatenate([np.cos(th * n), -np.sin(th * n)], axis=1)
    gt = ft.T / C
    return ft.astype(np.float32), gt.astype(np.float32)


def _gelu(x):
    c1 = 0.7978845608028654
    c2 = 0.7978845608028654 * 0.044715
    u = x * (c1 + c2 * (x * x))
    hx = 0.5 * x
    return hx + hx * jnp.tanh(u)


def _stats(x):
    m = jnp.mean(x, axis=0, keepdims=True)
    xc = x - m
    v = jnp.mean(xc * xc, axis=0, keepdims=True)
    return m, lax.rsqrt(v + EPS)


def _ln_cols(x):
    m = jnp.mean(x, axis=0, keepdims=True)
    xc = x - m
    v = jnp.mean(xc * xc, axis=0, keepdims=True)
    return xc * lax.rsqrt(v + EPS)


def _roll(x, s):
    return pltpu.bitcast(pltpu.roll(pltpu.bitcast(x, u32), s, axis=1), bf16)


def _dot(a, b):
    return jnp.dot(a, b, preferred_element_type=f32)


def _dot_nt(a, b):
    return lax.dot_general(a, b, (((1,), (1,)), ((), ())), preferred_element_type=f32)


def _kernel(q_hbm, k_hbm, v_hbm, sk_hbm, w1_hbm, w2_hbm, w3_hbm, w4_hbm,
            shift_hbm, dvec_hbm, gw_hbm, ft_hbm, gt_hbm,
            o_ref,
            q_v, k_v, v_v, qt_v, sk_v, w1_v, w2_v, w3_v, w4_v,
            shift_v, dvec_v, gw_v, ft_v, gt_v,
            w1t, w2t, h_v, x1_v, xn2_v, w3s, w4s, par_v, U, H, Z, sems, kv_sems, *gbufs):
    i = pl.program_id(0)

    def kv_copies(t):
        off = pl.multiple_of(t * TM, TM)
        return (pltpu.make_async_copy(k_hbm.at[:, pl.ds(pl.multiple_of(off - C, C), TM + C)],
                                      k_v.at[t % 2], kv_sems.at[0]),
                pltpu.make_async_copy(v_hbm.at[:, pl.ds(off, TM)], v_v.at[t % 2], kv_sems.at[1]))

    def w_copies(lo, n, s):
        return (pltpu.make_async_copy(w3_hbm.at[:, pl.ds(lo, n)], w3_v.at[:, pl.ds(lo, n)], sems.at[s]),
                pltpu.make_async_copy(w4_hbm.at[:, pl.ds(lo, n)], w4_v.at[:, pl.ds(lo, n)], sems.at[s + 1]))

    @pl.when(i == 0)
    def _first_step():
        cp_w1 = pltpu.make_async_copy(w1_hbm, w1_v, sems.at[0])
        cp_w2 = pltpu.make_async_copy(w2_hbm, w2_v, sems.at[1])
        cp_sk = pltpu.make_async_copy(sk_hbm, sk_v, sems.at[2])
        cp_small = [pltpu.make_async_copy(s, d, sems.at[5 + n]) for n, (s, d) in enumerate(
            ((gw_hbm, gw_v), (shift_hbm, shift_v), (dvec_hbm, dvec_v), (ft_hbm, ft_v), (gt_hbm, gt_v)))]
        cp_q = [pltpu.make_async_copy(q_hbm.at[:, pl.ds(lo, hi - lo)], q_v.at[:, pl.ds(lo, hi - lo)],
                                      sems.at[(10, 11, 14, 15)[n]])
                for n, (lo, hi) in enumerate(zip(QCUTS[:-1], QCUTS[1:]))]
        cp_wa = w_copies(0, PP, 12)
        cp_w3, cp_w4 = w_copies(PP, F - PP, 3)
        cp_w1.start()
        for c in cp_q:
            c.start()
        for c in cp_small:
            c.start()
        cp_w2.start()
        for c in cp_wa:
            c.start()
        cp_w4.start()
        cp_w3.start()
        cp_sk.start()
        cp_kv0 = (pltpu.make_async_copy(k_hbm.at[:, pl.ds(0, TM)], k_v.at[0, :, pl.ds(C, TM)],
                                        kv_sems.at[0]),
                  pltpu.make_async_copy(v_hbm.at[:, pl.ds(0, TM)], v_v.at[0], kv_sems.at[1]))
        for c in cp_kv0:
            c.start()
        cp_qt = [pltpu.make_async_copy(q_hbm.at[:, pl.ds(t * TM, TM)], qt_v.at[t], kv_sems.at[2])
                 for t in range(NSTEP)]

        h_v[:, 0:C] = jnp.zeros((D, C), bf16)
        h_v[:, C + S:] = jnp.zeros((D, C), bf16)
        k_v[0, :, 0:C] = jnp.zeros((D, C), bf16)
        Z[0:ZA] = jnp.zeros((ZA, D, 2 * C), f32)
        w3s[5, 0:8, 0:C] = jnp.zeros((8, C), u32)
        w4s[5, 0:8, 0:C] = jnp.zeros((8, C), u32)

        def stage_a(lo, n):
            if n % 512:
                acc = jnp.concatenate([_dot(w1t[0:DH, :], q_v[:, lo:lo + n]),
                                       _dot(w1t[DH:, :], q_v[:, lo:lo + n])], axis=0)
            else:
                acc = _dot(w1t[...], q_v[:, lo:lo + n])
            for c in range(n // C):
                m, r = _stats(q_v[:, lo + c * C:lo + (c + 1) * C].astype(f32))
                pre = (acc[:, c * C:(c + 1) * C] - par_v[6] * m) * r
                h_v[:, C + lo + c * C:C + lo + (c + 1) * C] = _gelu(pre).astype(bf16)

        def stage_b(b):
            lo = b * TB
            parts = []
            for gi, sh in enumerate((1, -1, 2, -2)):
                if sh > 0:
                    win = h_v[gi * G:(gi + 1) * G, lo:lo + TB + C]
                    parts.append(_roll(win, sh)[:, C:])
                else:
                    win = h_v[gi * G:(gi + 1) * G, C + lo:C + lo + TB + C]
                    parts.append(_roll(win, TB + C + sh)[:, :TB])
            hs_in = jnp.concatenate(parts, axis=0)
            x = q_v[:, lo:lo + TB].astype(f32)
            x1 = x + _dot(w2t[...], hs_in)
            for t in range(TB // TM):
                x1_v[lo // TM + t] = x1[:, t * TM:(t + 1) * TM]
            xn2_v[lo:lo + TB, :] = _ln_cols(x1).astype(bf16).T

        acts = {}

        def pp_up(b):
            lo = b * TB
            hb = TB // 2
            h3 = jnp.concatenate([_dot(xn2_v[lo:lo + hb, :], w3_v[:, 0:PP]),
                                  _dot(xn2_v[lo + hb:lo + TB, :], w3_v[:, 0:PP])], axis=0)
            acts[b] = _gelu(h3).astype(bf16)

        def pp_down(b):
            lo = b * TB
            p = _dot_nt(w4_v[:, 0:PP], acts.pop(b))
            for t in range(TB // TM):
                x1_v[lo // TM + t] = x1_v[lo // TM + t] + p[:, t * TM:(t + 1) * TM]

        def prep(src, dst, rh, c, lhs):
            lo = BOUNDS[c]
            for o in range(0, KH, C):
                def quad(rg, carry, o=o):
                    r1 = pl.ds(pl.multiple_of(rg * 16, 16), 16)
                    r2 = pl.ds(pl.multiple_of(rh + rg * 16, 16), 16)
                    c1 = slice(lo + o, lo + o + C)
                    c2 = slice(lo + KH + o, lo + KH + o + C)
                    t = dst[5, 0:8, 0:C]
                    m11 = pltpu.bitcast(pltpu.bitcast(src[r1, c1], u32) | t, bf16).astype(f32)
                    m22 = pltpu.bitcast(pltpu.bitcast(src[r2, c2], u32) | t, bf16).astype(f32)
                    m12 = src[r1, c2].astype(f32)
                    m21 = src[r2, c1].astype(f32)
                    if lhs:
                        ops = (m11 + m22, m21 + m22, m11 + m12, m21 - m11, m12 - m22)
                    else:
                        ops = (m11 + m22, m12 - m22, m21 - m11, m11 + m12, m21 + m22)
                    d0 = c * KH + o
                    rd = pl.ds(pl.multiple_of(rg * 8, 8), 8)
                    for n, op in enumerate(ops):
                        dst[i + n, rd, d0:d0 + C] = pltpu.bitcast(op.astype(bf16), u32)
                    return carry
                lax.fori_loop(0, rh // 16, quad, 0, unroll=True)

        def stage_h(j):
            H[j] = _dot(sk_v[:, j * C:(j + 1) * C], ft_v[...])

        def params():
            sh = shift_v[...].astype(f32)
            for j in range(4):
                par_v[j] = jnp.broadcast_to(sh[j:j + 1], (C, D)).T
            par_v[4] = jnp.broadcast_to(dvec_v[...].astype(f32).reshape(1, D), (C, D)).T
            par_v[5] = jnp.broadcast_to(gw_v[...].astype(f32).reshape(1, D), (C, D)).T

        cp_w1.wait()
        w1t[...] = w1_v[...].T
        Z[ZA:NP_ + 1] = jnp.zeros((NP_ + 1 - ZA, D, 2 * C), f32)
        for n, (lo, hi) in enumerate(zip(QCUTS[:-2], QCUTS[1:-1])):
            cp_q[n].wait()
            if n == 0:
                s1 = jnp.sum(w1_v[...].astype(f32), axis=0, keepdims=True)
                par_v[6] = jnp.broadcast_to(s1, (C, D)).T
            while lo < hi:
                n_ = (hi - lo) % 512 or 512
                stage_a(lo, n_)
                lo += n_
        for c in cp_small:
            c.wait()
        cp_w2.wait()
        cp_q[-1].wait()
        for c in cp_wa:
            c.wait()
        for c in cp_qt:
            c.start()
        w2t[...] = w2_v[...].T
        cnt = dict(a=0, b=0, u=0, d=0, h=0, p=0, q=0)
        fns = dict(a=lambda _: stage_a(QCUTS[-2], S - QCUTS[-2]), b=stage_b, u=pp_up, d=pp_down, h=stage_h,
                   p=lambda c: prep(w4_v, w4s, DH, c, True),
                   q=lambda c: prep(w3_v, w3s, KU, c, False))
        for tok in SEQ.split():
            if tok == 'W4':
                cp_w4.wait()
                params()
            elif tok == 'W3':
                cp_w3.wait()
                cp_sk.wait()
            else:
                for _ in range(int(tok[1:] or 1)):
                    fns[tok[0]](cnt[tok[0]])
                    cnt[tok[0]] += 1
        for c in list(cp_kv0) + cp_qt:
            c.wait()
        assert cnt == dict(a=1, b=S // TB, u=S // TB, d=S // TB, h=NC, p=NFS, q=NFS), cnt

    base = pl.multiple_of(i * TM, TM)

    @pl.when(i > 0)
    def _():
        for c in kv_copies(i):
            c.wait()

    @pl.when(i + 1 < NSTEP)
    def _():
        for c in kv_copies(i + 1):
            c.start()

    slot = i % 2
    zero = i // NSTEP

    kvd = []

    def conv_fwd():
        kwin = k_v[slot]
        shifted = [kwin[:, C:]] + [_roll(kwin, j)[:, C:] for j in range(1, 4)]
        for a in range(R):
            ks = shifted[0][:, a * C:(a + 1) * C].astype(f32) * par_v[0]
            for j in range(1, 4):
                ks = ks + shifted[j][:, a * C:(a + 1) * C].astype(f32) * par_v[j]
            kv = ks * v_v[slot, :, a * C:(a + 1) * C].astype(f32)
            kvd.append(kv * par_v[4])
            U[zero + a] = _dot(kv.astype(bf16), ft_v[...])

    def cmac(z, u, h):
        (ur, ui), (hr, hi) = u, h
        pr, pi = hr * ur - hi * ui, hr * ui + hi * ur
        return (pr, pi) if z is None else (z[0] + pr, z[1] + pi)

    lane = lax.broadcasted_iota(jnp.int32, (1, C), 1)
    sgn = (1 - 2 * (lane % 2)).astype(f32)

    def mac_one(r, rs):
        z = (Z[r, rs, :C], Z[r, rs, C:]) if r < NP_ else None
        for b in range(R):
            if r - b >= 0:
                z = cmac(z, (U[b, rs, :C], U[b, rs, C:]), (H[r - b, rs, :C], H[r - b, rs, C:]))
        return z

    def put(dst, rs, z):
        Z[zero + dst, rs, :C] = z[0]
        Z[zero + dst, rs, C:] = z[1]

    def conv_mac(rb, carry):
        rs = pl.ds(pl.multiple_of(rb * RB, RB), RB)
        yp = (Z[NP_, rs, :C], Z[NP_, rs, C:])
        for r in range(R):
            y = mac_one(r, rs)
            put(NP_ + 1 + r, rs, (y[0] - sgn * yp[1], y[1] + sgn * yp[0]))
            yp = y
        put(NP_, rs, yp)
        for r in range(R, NC):
            put(r - R, rs, mac_one(r, rs))
        return carry

    pre = []

    def conv_inv():
        for a in range(R):
            y = _dot(Z[NP_ + 1 + a].astype(bf16), gt_v[...])
            q = qt_v[i, :, a * C:(a + 1) * C].astype(f32)
            g = jax.nn.sigmoid(jnp.sum(q * par_v[5], axis=0, keepdims=True))
            og = 1.0 - g
            ga = (g * q) * (y + kvd[a])
            pre.append((ga + og * x1_v[i, :, a * C:(a + 1) * C], og))

    xn2 = xn2_v[pl.ds(base, TM), :]
    a11, a12, a21, a22 = xn2[:TH, :KU], xn2[:TH, KU:2 * KU], xn2[TH:, :KU], xn2[TH:, KU:2 * KU]
    f11, f12, f21, f22 = (t.astype(f32) for t in (a11, a12, a21, a22))
    xa = [(f11 + f22).astype(bf16), (f21 + f22).astype(bf16), a11, a22,
          (f11 + f12).astype(bf16), (f21 - f11).astype(bf16), (f12 - f22).astype(bf16)]
    xt = xn2[:, 2 * KU:]

    def up(c):
        lo, hi = BOUNDS[c], BOUNDS[c + 1]
        if c >= NFS:
            return _dot(xn2, w3_v[:, lo:hi])

        def bop(n):
            if n == 1:
                return w3_v[0:KU, lo:lo + KH]
            if n == 4:
                return w3_v[KU:2 * KU, lo + KH:hi]
            return pltpu.bitcast(w3s[{0: 0, 2: 1, 3: 2, 5: 3, 6: 4}[n], :, c * KH:(c + 1) * KH], bf16)

        m = {}
        for n in UP_ORDER:
            m[n] = _dot(xt, w3_v[2 * KU:, lo:hi]) if n == 't' else _dot(xa[n], bop(n))
        t = m['t']
        c21 = (t[TH:, :KH] + m[3]) + m[1]
        c12 = (t[:TH, KH:] + m[2]) + m[4]
        c11 = (((t[:TH, :KH] + m[3]) - m[4]) + m[0]) + m[6]
        c22 = (((t[TH:, KH:] - m[1]) + m[2]) + m[0]) + m[5]
        return c11, c12, c21, c22

    def act(c, h3):
        cs = slice((c % 2) * KH, (c % 2 + 1) * KH)
        c11, c12, c21, c22 = h3
        gb = gbufs[c // 2]
        gb[zero + 0, TH:, cs] = _gelu(c21)
        gb[zero + 1, :TH, cs] = _gelu(c12)
        gb[zero + 0, :TH, cs] = _gelu(c11)
        gb[zero + 1, TH:, cs] = _gelu(c22)

    accs = [None] * 7

    def down(g):
        gb = gbufs[g]
        b11, b12 = (lambda: gb[0, :TH]), (lambda: gb[0, TH:])
        b21, b22 = (lambda: gb[1, :TH]), (lambda: gb[1, TH:])
        tf = (lambda: b11() + b22(), b11, lambda: b12() - b22(), lambda: b21() - b11(), b22,
              lambda: b11() + b12(), lambda: b21() + b22())

        def aop(n):
            if n in (2, 3):
                rows = slice(0, DH) if n == 2 else slice(DH, D)
                o = 0 if n == 2 else KH
                return jnp.concatenate([w4_v[rows, BOUNDS[cc] + o:BOUNDS[cc] + o + KH]
                                        for cc in (2 * g, 2 * g + 1)], axis=1)
            return pltpu.bitcast(w4s[{0: 0, 1: 1, 4: 2, 5: 3, 6: 4}[n], :, g * TF:(g + 1) * TF], bf16)

        for n in DOWN_ORDER:
            m = _dot_nt(aop(n), tf[n]().astype(bf16))
            accs[n] = m if accs[n] is None else accs[n] + m

    extra = []
    h3 = up(0)
    for c in range(NF):
        h3n = up(c + 1) if c + 1 < NF else None
        if c == 0:
            conv_fwd()
            lax.fori_loop(0, NRB, conv_mac, 0, unroll=True)
        if c == CI:
            conv_inv()
        if c >= NFS:
            extra.append(_dot_nt(w4_v[:, BOUNDS[c]:BOUNDS[c + 1]], _gelu(h3).astype(bf16)))
        else:
            act(c, h3)
            if c % 2 == 1:
                down(c // 2)
        h3 = h3n

    m1, m2, m3, m4, m5, m6, m7 = accs
    acc = jnp.concatenate([
        jnp.concatenate([m1 + m4 - m5 + m7, m3 + m5], axis=1),
        jnp.concatenate([m2 + m4, m1 - m2 + m3 + m6], axis=1)], axis=0)
    for e in extra:
        acc = acc + e

    for a in range(R):
        pa, og = pre[a]
        o_ref[:, a * C:(a + 1) * C] = (pa + og * acc[:, a * C:(a + 1) * C]).astype(bf16)


_FT, _GT = _dft_mats()


@jax.jit
def pallas_gated_mix__ssm_conv_h3__mixer_s_mlp__prompt_kernel(
    A_q: jax.Array,
    A_k: jax.Array,
    A_v: jax.Array,
    A_shift_k: jax.Array,
    A_ssm_k: jax.Array,
    A_ssm_D: jax.Array,
    B_x: jax.Array,
    B_w1: jax.Array,
    B_w2: jax.Array,
    B_w3: jax.Array,
    B_w4: jax.Array,
    gate_w: jax.Array,
):
    del B_x
    hbm = pl.BlockSpec(memory_space=pltpu.MemorySpace.HBM)
    out_t = pl.pallas_call(
        _kernel,
        grid=(NSTEP,),
        in_specs=[hbm] * 13,
        out_specs=pl.BlockSpec((D, TM), lambda i: (0, i)),
        out_shape=jax.ShapeDtypeStruct((D, S), bf16),
        scratch_shapes=[
            pltpu.VMEM((D, S), bf16),
            pltpu.VMEM((2, D, C + TM), bf16),
            pltpu.VMEM((2, D, TM), bf16),
            pltpu.VMEM((NSTEP, D, TM), bf16),
            pltpu.VMEM((D, S), bf16),
            pltpu.VMEM((D, D), bf16),
            pltpu.VMEM((D, D), bf16),
            pltpu.VMEM((D, F), bf16),
            pltpu.VMEM((D, F), bf16),
            pltpu.VMEM((4, D), bf16),
            pltpu.VMEM((D,), bf16),
            pltpu.VMEM((D,), bf16),
            pltpu.VMEM((C, 2 * C), bf16),
            pltpu.VMEM((2 * C, C), bf16),
            pltpu.VMEM((D, D), bf16),
            pltpu.VMEM((D, D), bf16),
            pltpu.VMEM((D, S + 2 * C), bf16),
            pltpu.VMEM((NSTEP, D, TM), f32),
            pltpu.VMEM((S, D), bf16),
            pltpu.VMEM((6, KU // 2, NFS * KH), u32),
            pltpu.VMEM((6, DH // 2, NFS * KH), u32),
            pltpu.VMEM((7, D, C), f32),
            pltpu.VMEM((R, D, 2 * C), f32),
            pltpu.VMEM((NC, D, 2 * C), f32),
            pltpu.VMEM((NC + 1, D, 2 * C), f32),
            pltpu.SemaphoreType.DMA((16,)),
            pltpu.SemaphoreType.DMA((3,)),
        ] + [pltpu.VMEM((2, TM, TF), f32)] * NG,
        compiler_params=pltpu.CompilerParams(
            dimension_semantics=("arbitrary",),
            vmem_limit_bytes=110 * 1024 * 1024,
            disable_bounds_checks=True),
    )(A_q[0].T, A_k[0].T, A_v[0].T, A_ssm_k, B_w1, B_w2, B_w3, B_w4.T,
      A_shift_k.T, A_ssm_D, gate_w,
      jnp.asarray(_FT, bf16), jnp.asarray(_GT, bf16))
    return out_t.T[None]
```

```python
import numpy as np
import jax
import jax.numpy as jnp
from jax import lax
import jax.experimental.pallas as pl
import jax.experimental.pallas.tpu as pltpu

S, D, F = 2048, 576, 4608
C = 128
NC = S // C
G = D // 4
EPS = 1e-5
f32 = jnp.float32
bf16 = jnp.bfloat16
u32 = jnp.uint32

TM = 256
TB = 512
TF = 512
PP = 256
RB = 16
ZA = 13
NSTEP = S // TM
R = TM // C
NRB = D // RB
BOUNDS = list(range(PP, F, TF)) + [F]
NF = len(BOUNDS) - 1
DH = D // 2
TH = TM // 2
NG = (F - PP) // (2 * TF)
NFS = 2 * NG
KH = TF // 2
KU = 2 * C
NP_ = NC - R
QCUTS = [0, 256, 768, 1280, S]
SEQ = "a b b u W4 p1 d p3 b u p1 d p3 b u d W3 q4 h8 u q4 h8 d"
UP_ORDER = (2, 't', 4, 3, 1, 0, 6, 5)
DOWN_ORDER = (1, 3, 2, 4, 0, 6, 5)
CI = 7


def _dft_mats():
    n = np.arange(C)[:, None].astype(np.float64)
    th = 2.0 * np.pi * (np.arange(C)[None, :] + 0.5) / (2 * C)
    ft = np.concatenate([np.cos(th * n), -np.sin(th * n)], axis=1)
    gt = ft.T / C
    return ft.astype(np.float32), gt.astype(np.float32)


def _gelu2(h):
    c1 = 2.0 * 0.7978845608028654
    c2 = 8.0 * 0.7978845608028654 * 0.044715
    return h + h * jnp.tanh(h * (c1 + c2 * (h * h)))


def _stats_half(x):
    m = jnp.mean(x, axis=0, keepdims=True)
    xc = x - m
    v = jnp.mean(xc * xc, axis=0, keepdims=True)
    return m, 0.5 * lax.rsqrt(v + EPS)


def _ln_half(x):
    m = jnp.mean(x, axis=0, keepdims=True)
    xc = x - m
    v = jnp.mean(xc * xc, axis=0, keepdims=True)
    return xc * (0.5 * lax.rsqrt(v + EPS))


def _roll(x, s):
    return pltpu.bitcast(pltpu.roll(pltpu.bitcast(x, u32), s, axis=1), bf16)


def _dot(a, b):
    return jnp.dot(a, b, preferred_element_type=f32)


def _dot_nt(a, b):
    return lax.dot_general(a, b, (((1,), (1,)), ((), ())), preferred_element_type=f32)


def _kernel(q_hbm, k_hbm, v_hbm, sk_hbm, w1_hbm, w2_hbm, w3_hbm, w4_hbm,
            shift_hbm, dvec_hbm, gw_hbm, ft_hbm, gt_hbm,
            o_ref,
            q_v, k_v, v_v, qt_v, sk_v, w1_v, w2_v, w3_v, w4_v,
            shift_v, dvec_v, gw_v, ft_v, gt_v,
            w1t, w2t, h_v, x1_v, xn2_v, w3s, w4s, par_v, U, H, Z, sems, kv_sems, *gbufs):
    i = pl.program_id(0)

    def kv_copies(t):
        off = pl.multiple_of(t * TM, TM)
        return (pltpu.make_async_copy(k_hbm.at[:, pl.ds(pl.multiple_of(off - C, C), TM + C)],
                                      k_v.at[t % 2], kv_sems.at[0]),
                pltpu.make_async_copy(v_hbm.at[:, pl.ds(off, TM)], v_v.at[t % 2], kv_sems.at[1]))

    def w_copies(lo, n, s):
        return (pltpu.make_async_copy(w3_hbm.at[:, pl.ds(lo, n)], w3_v.at[:, pl.ds(lo, n)], sems.at[s]),
                pltpu.make_async_copy(w4_hbm.at[:, pl.ds(lo, n)], w4_v.at[:, pl.ds(lo, n)], sems.at[s + 1]))

    @pl.when(i == 0)
    def _first_step():
        cp_w1 = pltpu.make_async_copy(w1_hbm, w1_v, sems.at[0])
        cp_w2 = pltpu.make_async_copy(w2_hbm, w2_v, sems.at[1])
        cp_sk = pltpu.make_async_copy(sk_hbm, sk_v, sems.at[2])
        cp_small = [pltpu.make_async_copy(s, d, sems.at[5 + n]) for n, (s, d) in enumerate(
            ((gw_hbm, gw_v), (shift_hbm, shift_v), (dvec_hbm, dvec_v), (ft_hbm, ft_v), (gt_hbm, gt_v)))]
        cp_q = [pltpu.make_async_copy(q_hbm.at[:, pl.ds(lo, hi - lo)], q_v.at[:, pl.ds(lo, hi - lo)],
                                      sems.at[(10, 11, 14, 15)[n]])
                for n, (lo, hi) in enumerate(zip(QCUTS[:-1], QCUTS[1:]))]
        cp_wa = w_copies(0, PP, 12)
        cp_w3, cp_w4 = w_copies(PP, F - PP, 3)
        cp_w1.start()
        for c in cp_q:
            c.start()
        for c in cp_small:
            c.start()
        cp_w2.start()
        for c in cp_wa:
            c.start()
        cp_w4.start()
        cp_w3.start()
        cp_sk.start()
        cp_kv0 = (pltpu.make_async_copy(k_hbm.at[:, pl.ds(0, TM)], k_v.at[0, :, pl.ds(C, TM)],
                                        kv_sems.at[0]),
                  pltpu.make_async_copy(v_hbm.at[:, pl.ds(0, TM)], v_v.at[0], kv_sems.at[1]))
        for c in cp_kv0:
            c.start()
        cp_qt = [pltpu.make_async_copy(q_hbm.at[:, pl.ds(t * TM, TM)], qt_v.at[t], kv_sems.at[2])
                 for t in range(NSTEP)]

        h_v[:, 0:C] = jnp.zeros((D, C), bf16)
        h_v[:, C + S:] = jnp.zeros((D, C), bf16)
        k_v[0, :, 0:C] = jnp.zeros((D, C), bf16)
        Z[0:ZA] = jnp.zeros((ZA, D, 2 * C), f32)
        w3s[5, 0:8, 0:C] = jnp.zeros((8, C), u32)
        w4s[5, 0:8, 0:C] = jnp.zeros((8, C), u32)

        def stage_a(lo, n):
            if n % 512:
                acc = jnp.concatenate([_dot(w1t[0:DH, :], q_v[:, lo:lo + n]),
                                       _dot(w1t[DH:, :], q_v[:, lo:lo + n])], axis=0)
            else:
                acc = _dot(w1t[...], q_v[:, lo:lo + n])
            for c in range(n // C):
                m, r = _stats_half(q_v[:, lo + c * C:lo + (c + 1) * C].astype(f32))
                pre = (acc[:, c * C:(c + 1) * C] - par_v[6] * m) * r
                h_v[:, C + lo + c * C:C + lo + (c + 1) * C] = _gelu2(pre).astype(bf16)

        def stage_b(b):
            lo = b * TB
            parts = []
            for gi, sh in enumerate((1, -1, 2, -2)):
                if sh > 0:
                    win = h_v[gi * G:(gi + 1) * G, lo:lo + TB + C]
                    parts.append(_roll(win, sh)[:, C:])
                else:
                    win = h_v[gi * G:(gi + 1) * G, C + lo:C + lo + TB + C]
                    parts.append(_roll(win, TB + C + sh)[:, :TB])
            hs_in = jnp.concatenate(parts, axis=0)
            x = q_v[:, lo:lo + TB].astype(f32)
            x1 = x + _dot(w2t[...], hs_in)
            for t in range(TB // TM):
                x1_v[lo // TM + t] = x1[:, t * TM:(t + 1) * TM]
            xn2_v[lo:lo + TB, :] = _ln_half(x1).astype(bf16).T

        acts = {}

        def pp_up(b):
            lo = b * TB
            hb = TB // 2
            h3 = jnp.concatenate([_dot(xn2_v[lo:lo + hb, :], w3_v[:, 0:PP]),
                                  _dot(xn2_v[lo + hb:lo + TB, :], w3_v[:, 0:PP])], axis=0)
            acts[b] = _gelu2(h3).astype(bf16)

        def pp_down(b):
            lo = b * TB
            p = _dot_nt(w4_v[:, 0:PP], acts.pop(b))
            for t in range(TB // TM):
                x1_v[lo // TM + t] = x1_v[lo // TM + t] + p[:, t * TM:(t + 1) * TM]

        def prep(src, dst, rh, c, lhs):
            lo = BOUNDS[c]
            for o in range(0, KH, C):
                def quad(rg, carry, o=o):
                    r1 = pl.ds(pl.multiple_of(rg * 16, 16), 16)
                    r2 = pl.ds(pl.multiple_of(rh + rg * 16, 16), 16)
                    c1 = slice(lo + o, lo + o + C)
                    c2 = slice(lo + KH + o, lo + KH + o + C)
                    t = dst[5, 0:8, 0:C]
                    m11 = pltpu.bitcast(pltpu.bitcast(src[r1, c1], u32) | t, bf16).astype(f32)
                    m22 = pltpu.bitcast(pltpu.bitcast(src[r2, c2], u32) | t, bf16).astype(f32)
                    m12 = src[r1, c2].astype(f32)
                    m21 = src[r2, c1].astype(f32)
                    if lhs:
                        ops = (m11 + m22, m21 + m22, m11 + m12, m21 - m11, m12 - m22)
                    else:
                        ops = (m11 + m22, m12 - m22, m21 - m11, m11 + m12, m21 + m22)
                    d0 = c * KH + o
                    rd = pl.ds(pl.multiple_of(rg * 8, 8), 8)
                    for n, op in enumerate(ops):
                        dst[i + n, rd, d0:d0 + C] = pltpu.bitcast(op.astype(bf16), u32)
                    return carry
                lax.fori_loop(0, rh // 16, quad, 0, unroll=True)

        def stage_h(j):
            H[j] = _dot(sk_v[:, j * C:(j + 1) * C], ft_v[...])

        def params():
            sh = shift_v[...].astype(f32)
            for j in range(4):
                par_v[j] = jnp.broadcast_to(sh[j:j + 1], (C, D)).T
            par_v[4] = jnp.broadcast_to(dvec_v[...].astype(f32).reshape(1, D), (C, D)).T
            par_v[5] = jnp.broadcast_to(gw_v[...].astype(f32).reshape(1, D), (C, D)).T

        cp_w1.wait()
        w1t[...] = w1_v[...].T
        Z[ZA:NP_ + 1] = jnp.zeros((NP_ + 1 - ZA, D, 2 * C), f32)
        for n, (lo, hi) in enumerate(zip(QCUTS[:-2], QCUTS[1:-1])):
            cp_q[n].wait()
            if n == 0:
                s1 = jnp.sum(w1_v[...].astype(f32), axis=0, keepdims=True)
                par_v[6] = jnp.broadcast_to(s1, (C, D)).T
            while lo < hi:
                n_ = (hi - lo) % 512 or 512
                stage_a(lo, n_)
                lo += n_
        for c in cp_small:
            c.wait()
        cp_w2.wait()
        cp_q[-1].wait()
        for c in cp_wa:
            c.wait()
        for c in cp_qt:
            c.start()
        w2t[...] = w2_v[...].T
        cnt = dict(a=0, b=0, u=0, d=0, h=0, p=0, q=0)
        fns = dict(a=lambda _: stage_a(QCUTS[-2], S - QCUTS[-2]), b=stage_b, u=pp_up, d=pp_down, h=stage_h,
                   p=lambda c: prep(w4_v, w4s, DH, c, True),
                   q=lambda c: prep(w3_v, w3s, KU, c, False))
        for tok in SEQ.split():
            if tok == 'W4':
                cp_w4.wait()
                params()
            elif tok == 'W3':
                cp_w3.wait()
                cp_sk.wait()
            else:
                for _ in range(int(tok[1:] or 1)):
                    fns[tok[0]](cnt[tok[0]])
                    cnt[tok[0]] += 1
        for c in list(cp_kv0) + cp_qt:
            c.wait()
        assert cnt == dict(a=1, b=S // TB, u=S // TB, d=S // TB, h=NC, p=NFS, q=NFS), cnt

    base = pl.multiple_of(i * TM, TM)

    @pl.when(i > 0)
    def _():
        for c in kv_copies(i):
            c.wait()

    @pl.when(i + 1 < NSTEP)
    def _():
        for c in kv_copies(i + 1):
            c.start()

    slot = i % 2
    zero = i // NSTEP

    kvd = []

    def conv_fwd():
        kwin = k_v[slot]
        shifted = [kwin[:, C:]] + [_roll(kwin, j)[:, C:] for j in range(1, 4)]
        for a in range(R):
            ks = shifted[0][:, a * C:(a + 1) * C].astype(f32) * par_v[0]
            for j in range(1, 4):
                ks = ks + shifted[j][:, a * C:(a + 1) * C].astype(f32) * par_v[j]
            kv = ks * v_v[slot, :, a * C:(a + 1) * C].astype(f32)
            kvd.append(kv * par_v[4])
            U[zero + a] = _dot(kv.astype(bf16), ft_v[...])

    def cmac(z, u, h):
        (ur, ui), (hr, hi) = u, h
        pr, pi = hr * ur - hi * ui, hr * ui + hi * ur
        return (pr, pi) if z is None else (z[0] + pr, z[1] + pi)

    lane = lax.broadcasted_iota(jnp.int32, (1, C), 1)
    sgn = (1 - 2 * (lane % 2)).astype(f32)

    def mac_one(r, rs):
        z = (Z[r, rs, :C], Z[r, rs, C:]) if r < NP_ else None
        for b in range(R):
            if r - b >= 0:
                z = cmac(z, (U[b, rs, :C], U[b, rs, C:]), (H[r - b, rs, :C], H[r - b, rs, C:]))
        return z

    def put(dst, rs, z):
        Z[zero + dst, rs, :C] = z[0]
        Z[zero + dst, rs, C:] = z[1]

    def conv_mac(rb, carry):
        rs = pl.ds(pl.multiple_of(rb * RB, RB), RB)
        yp = (Z[NP_, rs, :C], Z[NP_, rs, C:])
        for r in range(R):
            y = mac_one(r, rs)
            put(NP_ + 1 + r, rs, (y[0] - sgn * yp[1], y[1] + sgn * yp[0]))
            yp = y
        put(NP_, rs, yp)
        for r in range(R, NC):
            put(r - R, rs, mac_one(r, rs))
        return carry

    pre = []

    def conv_inv():
        for a in range(R):
            y = _dot(Z[NP_ + 1 + a].astype(bf16), gt_v[...])
            q = qt_v[i, :, a * C:(a + 1) * C].astype(f32)
            g = jax.nn.sigmoid(jnp.sum(q * par_v[5], axis=0, keepdims=True))
            og = 1.0 - g
            ga = (g * q) * (y + kvd[a])
            pre.append((ga + og * x1_v[i, :, a * C:(a + 1) * C], og))

    xn2 = xn2_v[pl.ds(base, TM), :]
    a11, a12, a21, a22 = xn2[:TH, :KU], xn2[:TH, KU:2 * KU], xn2[TH:, :KU], xn2[TH:, KU:2 * KU]
    f11, f12, f21, f22 = (t.astype(f32) for t in (a11, a12, a21, a22))
    xa = [(f11 + f22).astype(bf16), (f21 + f22).astype(bf16), a11, a22,
          (f11 + f12).astype(bf16), (f21 - f11).astype(bf16), (f12 - f22).astype(bf16)]
    xt = xn2[:, 2 * KU:]

    def up(c):
        lo, hi = BOUNDS[c], BOUNDS[c + 1]
        if c >= NFS:
            return _dot(xn2, w3_v[:, lo:hi])

        def bop(n):
            if n == 1:
                return w3_v[0:KU, lo:lo + KH]
            if n == 4:
                return w3_v[KU:2 * KU, lo + KH:hi]
            return pltpu.bitcast(w3s[{0: 0, 2: 1, 3: 2, 5: 3, 6: 4}[n], :, c * KH:(c + 1) * KH], bf16)

        m = {}
        for n in UP_ORDER:
            m[n] = _dot(xt, w3_v[2 * KU:, lo:hi]) if n == 't' else _dot(xa[n], bop(n))
        t = m['t']
        c21 = (t[TH:, :KH] + m[3]) + m[1]
        c12 = (t[:TH, KH:] + m[2]) + m[4]
        c11 = (((t[:TH, :KH] + m[3]) - m[4]) + m[0]) + m[6]
        c22 = (((t[TH:, KH:] - m[1]) + m[2]) + m[0]) + m[5]
        return c11, c12, c21, c22

    def act(c, h3):
        cs = slice((c % 2) * KH, (c % 2 + 1) * KH)
        c11, c12, c21, c22 = h3
        gb = gbufs[c // 2]
        gb[zero + 0, TH:, cs] = _gelu2(c21)
        gb[zero + 1, :TH, cs] = _gelu2(c12)
        gb[zero + 0, :TH, cs] = _gelu2(c11)
        gb[zero + 1, TH:, cs] = _gelu2(c22)

    accs = [None] * 7

    def down(g):
        gb = gbufs[g]
        b11, b12 = (lambda: gb[0, :TH]), (lambda: gb[0, TH:])
        b21, b22 = (lambda: gb[1, :TH]), (lambda: gb[1, TH:])
        tf = (lambda: b11() + b22(), b11, lambda: b12() - b22(), lambda: b21() - b11(), b22,
              lambda: b11() + b12(), lambda: b21() + b22())

        def aop(n):
            if n in (2, 3):
                rows = slice(0, DH) if n == 2 else slice(DH, D)
                o = 0 if n == 2 else KH
                return jnp.concatenate([w4_v[rows, BOUNDS[cc] + o:BOUNDS[cc] + o + KH]
                                        for cc in (2 * g, 2 * g + 1)], axis=1)
            return pltpu.bitcast(w4s[{0: 0, 1: 1, 4: 2, 5: 3, 6: 4}[n], :, g * TF:(g + 1) * TF], bf16)

        for n in DOWN_ORDER:
            m = _dot_nt(aop(n), tf[n]().astype(bf16))
            accs[n] = m if accs[n] is None else accs[n] + m

    extra = []
    h3 = up(0)
    for c in range(NF):
        h3n = up(c + 1) if c + 1 < NF else None
        if c == 0:
            conv_fwd()
            lax.fori_loop(0, NRB, conv_mac, 0, unroll=True)
        if c == CI:
            conv_inv()
        if c >= NFS:
            extra.append(_dot_nt(w4_v[:, BOUNDS[c]:BOUNDS[c + 1]], _gelu2(h3).astype(bf16)))
        else:
            act(c, h3)
            if c % 2 == 1:
                down(c // 2)
        h3 = h3n

    m1, m2, m3, m4, m5, m6, m7 = accs
    acc = jnp.concatenate([
        jnp.concatenate([m1 + m4 - m5 + m7, m3 + m5], axis=1),
        jnp.concatenate([m2 + m4, m1 - m2 + m3 + m6], axis=1)], axis=0)
    for e in extra:
        acc = acc + e

    for a in range(R):
        pa, og = pre[a]
        o_ref[:, a * C:(a + 1) * C] = (pa + og * acc[:, a * C:(a + 1) * C]).astype(bf16)


_FT, _GT = _dft_mats()


@jax.jit
def pallas_gated_mix__ssm_conv_h3__mixer_s_mlp__prompt_kernel(
    A_q: jax.Array,
    A_k: jax.Array,
    A_v: jax.Array,
    A_shift_k: jax.Array,
    A_ssm_k: jax.Array,
    A_ssm_D: jax.Array,
    B_x: jax.Array,
    B_w1: jax.Array,
    B_w2: jax.Array,
    B_w3: jax.Array,
    B_w4: jax.Array,
    gate_w: jax.Array,
):
    del B_x
    hbm = pl.BlockSpec(memory_space=pltpu.MemorySpace.HBM)
    out_t = pl.pallas_call(
        _kernel,
        grid=(NSTEP,),
        in_specs=[hbm] * 13,
        out_specs=pl.BlockSpec((D, TM), lambda i: (0, i)),
        out_shape=jax.ShapeDtypeStruct((D, S), bf16),
        scratch_shapes=[
            pltpu.VMEM((D, S), bf16),
            pltpu.VMEM((2, D, C + TM), bf16),
            pltpu.VMEM((2, D, TM), bf16),
            pltpu.VMEM((NSTEP, D, TM), bf16),
            pltpu.VMEM((D, S), bf16),
            pltpu.VMEM((D, D), bf16),
            pltpu.VMEM((D, D), bf16),
            pltpu.VMEM((D, F), bf16),
            pltpu.VMEM((D, F), bf16),
            pltpu.VMEM((4, D), bf16),
            pltpu.VMEM((D,), bf16),
            pltpu.VMEM((D,), bf16),
            pltpu.VMEM((C, 2 * C), bf16),
            pltpu.VMEM((2 * C, C), bf16),
            pltpu.VMEM((D, D), bf16),
            pltpu.VMEM((D, D), bf16),
            pltpu.VMEM((D, S + 2 * C), bf16),
            pltpu.VMEM((NSTEP, D, TM), f32),
            pltpu.VMEM((S, D), bf16),
            pltpu.VMEM((6, KU // 2, NFS * KH), u32),
            pltpu.VMEM((6, DH // 2, NFS * KH), u32),
            pltpu.VMEM((7, D, C), f32),
            pltpu.VMEM((R, D, 2 * C), f32),
            pltpu.VMEM((NC, D, 2 * C), f32),
            pltpu.VMEM((NC + 1, D, 2 * C), f32),
            pltpu.SemaphoreType.DMA((16,)),
            pltpu.SemaphoreType.DMA((3,)),
        ] + [pltpu.VMEM((2, TM, TF), f32)] * NG,
        compiler_params=pltpu.CompilerParams(
            dimension_semantics=("arbitrary",),
            vmem_limit_bytes=110 * 1024 * 1024,
            disable_bounds_checks=True),
    )(A_q[0].T, A_k[0].T, A_v[0].T, A_ssm_k, B_w1, B_w2, B_w3, B_w4.T,
      A_shift_k.T, A_ssm_D, gate_w,
      jnp.asarray(_FT, bf16), jnp.asarray(_GT, bf16))
    return out_t.T[None]
```
